```python
import os as _os
_os.environ.setdefault("JAX_PLATFORMS", "cpu")
import jax
import jax.numpy as jnp

def _softmax(x, axis=-1):
    return jax.nn.softmax(x, axis=axis)
def _gelu(x):
    return jax.nn.gelu(x, approximate=True)
def _silu(x):
    return jax.nn.silu(x)
def _sigmoid(x):
    return jax.nn.sigmoid(x)
def _layernorm(x, axis=-1, eps=1e-5):
    m = jnp.mean(x, axis=axis, keepdims=True)
    v = jnp.var(x, axis=axis, keepdims=True)
    return (x - m) / jnp.sqrt(v + eps)
def _scatter_add(tgt, idx, src, axis=0):
    return tgt.at[idx].add(src)
def _segment_sum(src, seg, n):
    return jax.ops.segment_sum(src, seg, n)
class _Rng:
    def __init__(self, key):
        self._k = key
    def _next(self):
        self._k, sub = jax.random.split(self._k)
        return sub
    def normal(self, shape):
        return jax.random.normal(self._next(), shape, dtype=jnp.bfloat16)
    def randint(self, lo, hi, shape):
        return jax.random.randint(self._next(), shape, lo, hi, dtype=jnp.int32)
    def uniform(self, shape, lo=0.0, hi=1.0):
        return jax.random.uniform(self._next(), shape, jnp.bfloat16, lo, hi)
    def permutation(self, n):
        return jax.random.permutation(self._next(), n)


kernel_name = 'parallel_sum__sliding_block_cached__dense_activation_mish__decode'

def setup_inputs():
    _rng = _Rng(jax.random.key(int.from_bytes(__import__("os").urandom(4), "little")))
    _w = (lambda a: (lambda t: t.astype(jnp.bfloat16) if jnp.issubdtype(t.dtype, jnp.floating) else t)(jnp.asarray(a)))
    def _A_setup():
        B, Sq, D = 2, 1, 512
        Hq, Hkv, Sk, Dh = 32, 8, 32768, 128
        assert Hq % Hkv == 0, (Hq, Hkv)
        return {
            "x": _w((lambda *s: _rng.normal(s) * 0.05)(B, Sq, D)),
            "k_cache": _w((lambda *s: _rng.normal(s) * 0.8)(B, Hkv, Sk, Dh)),
            "v_cache": _w((lambda *s: _rng.normal(s) * 0.8)(B, Hkv, Sk, Dh)),
            "wq": _w((lambda *s: _rng.normal(s) * 0.8)(D, Hq * Dh) * (D ** -0.5)),
            "wo": _w((lambda *s: _rng.normal(s) * 0.8)(Hq * Dh, D) * ((Hq * Dh) ** -0.5)),
        }
    _A_in = _A_setup()

    def _B_setup():
        B, S, D, F = 2, 1, 512, 1792
        return {
            "x": _w((lambda *s: _rng.normal(s) * 0.05)(B, S, D)),
            "w1": _w((lambda *s: _rng.normal(s) * 0.4)(D, F) * (D ** -0.5)),
            "b1": _w((lambda *s: _rng.normal(s) * 0.05)(F)),
            "w2": _w((lambda *s: _rng.normal(s) * 0.05)(F, D) * (F ** -0.5)),
        }
    _B_in = _B_setup()

    return {
        "A_x": _A_in["x"],
        "A_k_cache": _A_in["k_cache"],
        "A_v_cache": _A_in["v_cache"],
        "A_wq": _A_in["wq"],
        "A_wo": _A_in["wo"],
        "B_x": _B_in["x"],
        "B_w1": _B_in["w1"],
        "B_b1": _B_in["b1"],
        "B_w2": _B_in["w2"],
    }

def reference(A_x, A_k_cache, A_v_cache, A_wq, A_wo, B_x, B_w1, B_b1, B_w2):
    def _A_ref(x, k_cache, v_cache, wq, wo):
        B, Sq, D = x.shape
        Hq, Dh = 32, 128
        Hkv, Sk = k_cache.shape[1], k_cache.shape[2]
        W = min(4096, max(256, Sk // 4))
        rep = Hq // Hkv
        q = (lambda x, *d: x.transpose(*d))((x @ wq).reshape(B, Sq, Hq, Dh), 0, 2, 1, 3)
        k = jnp.repeat(k_cache[:, :, Sk - W:, :], rep, axis=1)
        v = jnp.repeat(v_cache[:, :, Sk - W:, :], rep, axis=1)
        scores = jnp.einsum("bhqd,bhkd->bhqk", q, k) * (Dh ** -0.5)
        p = _softmax(scores, axis=-1)
        o = jnp.einsum("bhqk,bhkd->bhqd", p, v)
        return (lambda x, *d: x.transpose(*d))(o, 0, 2, 1, 3).reshape(B, Sq, Hq * Dh) @ wo

    def _B_ref(x, w1, b1, w2):
        h = jnp.einsum("bsd,df->bsf", x, w1) + b1
        sp = jnp.log1p(jnp.exp(-jnp.abs(h))) + jnp.where(h > 0, h, jnp.zeros_like(h))
        act = h * jnp.tanh(sp)
        return jnp.einsum("bsf,fd->bsd", act, w2)

    x = A_x
    xn = _layernorm(x, axis=-1)
    return x + _A_ref(xn, A_k_cache, A_v_cache, A_wq, A_wo) + _B_ref(xn, B_w1, B_b1, B_w2)
```

```python
import jax, jax.numpy as jnp
from jax import lax
from jax.experimental import pallas as pl
from jax.experimental.pallas import tpu as pltpu

B, D = 2, 512
HQ, HKV, DH = 32, 8, 128
REP = HQ // HKV
F = 1792
NT = (((1,), (1,)), ((), ()))
UNROLL = False

def make_kernel(W, SK):
    def kernel(x_hbm, k_hbm, v_hbm, wq_hbm, wo_hbm, w1_hbm, b1_hbm, w2_hbm, o_ref,
               xbuf, b1buf, kbuf, vbuf, wqb, wob, w1b, w2b, qscr, sems):
        def ck(h):
            return pltpu.make_async_copy(k_hbm.at[:, h, pl.ds(SK - W, W), :], kbuf.at[h], sems.at[0])
        def cv(h):
            return pltpu.make_async_copy(v_hbm.at[:, h, pl.ds(SK - W, W), :], vbuf.at[h], sems.at[1])
        def cwo(h):
            return pltpu.make_async_copy(wo_hbm.at[pl.ds(h * 512, 512), :], wob.at[h], sems.at[2])
        cx = pltpu.make_async_copy(x_hbm, xbuf, sems.at[3])
        cb1 = pltpu.make_async_copy(b1_hbm, b1buf, sems.at[3])
        cwq = pltpu.make_async_copy(wq_hbm, wqb, sems.at[3])
        cw1 = pltpu.make_async_copy(w1_hbm, w1b, sems.at[4])
        cw2 = pltpu.make_async_copy(w2_hbm, w2b, sems.at[3])
        cx.start(); cb1.start(); cwq.start(); cw1.start()
        ck(0).start(); cv(0).start(); cwo(0).start()
        cx.wait(); cb1.wait(); cwq.wait()

        row = lax.broadcasted_iota(jnp.int32, (8, D), 0)
        xx = xbuf[...].astype(jnp.float32)
        x0 = xx[0:1]
        x1 = xx[1:2]
        x8 = jnp.where(row < 4, jnp.broadcast_to(x0, (8, D)), jnp.broadcast_to(x1, (8, D)))
        mu = jnp.mean(x8, axis=-1, keepdims=True)
        xc = x8 - mu
        var = jnp.mean(xc * xc, axis=-1, keepdims=True)
        xn8 = xc / jnp.sqrt(var + 1e-5)
        xn8b = xn8.astype(jnp.bfloat16)
        row128 = lax.broadcasted_iota(jnp.int32, (8, DH), 0)
        rowW = lax.broadcasted_iota(jnp.int32, (8, W), 0)
        scale = DH ** -0.5
        qall = jnp.dot(xn8b, wqb[...], preferred_element_type=jnp.float32)
        for h in range(HKV):
            q = qall[:, (4 * h) * 128:(4 * h + 1) * 128]
            for j in range(1, REP):
                q = jnp.where(row128 % 4 == j, qall[:, (4 * h + j) * 128:(4 * h + j + 1) * 128], q)
            qscr[h] = q
        cw1.wait()
        hh = jnp.dot(xn8b, w1b[...], preferred_element_type=jnp.float32) + b1buf[...].astype(jnp.float32)[None, :]
        sp = jnp.log1p(jnp.exp(-jnp.abs(hh))) + jnp.maximum(hh, 0.0)
        act = (hh * jnp.tanh(sp)).astype(jnp.bfloat16)

        def head(h, acc, last=False):
            qb = qscr[h].astype(jnp.bfloat16)
            ck(h).wait()
            if not last: ck(h + 1).start()
            else: cw2.start()
            s0 = lax.dot_general(qb, kbuf[h, 0], NT, preferred_element_type=jnp.float32)
            s1 = lax.dot_general(qb, kbuf[h, 1], NT, preferred_element_type=jnp.float32)
            s = jnp.where(rowW < 4, s0, s1) * scale
            m = jnp.max(s, axis=-1, keepdims=True)
            p = jnp.exp(s - m)
            l = jnp.sum(p, axis=-1, keepdims=True)
            pb = p.astype(jnp.bfloat16)
            cv(h).wait()
            if not last: cv(h + 1).start()
            o0 = jnp.dot(pb, vbuf[h, 0], preferred_element_type=jnp.float32)
            o1 = jnp.dot(pb, vbuf[h, 1], preferred_element_type=jnp.float32)
            o = jnp.where(row128 < 4, o0, o1) / l
            cwo(h).wait()
            if not last: cwo(h + 1).start()
            for j in range(REP):
                oj = jnp.where(row128 % 4 == j, o, 0.0).astype(jnp.bfloat16)
                acc = acc + jnp.dot(oj, wob[h, j * 128:(j + 1) * 128, :], preferred_element_type=jnp.float32)
            return acc

        acc = jnp.zeros((8, D), jnp.float32)
        if UNROLL:
            for h in range(HKV - 1):
                acc = head(h, acc)
        else:
            acc = lax.fori_loop(0, HKV - 1, head, acc)
        acc = head(HKV - 1, acc, last=True)
        a0 = jnp.sum(acc[0:4], axis=0, keepdims=True)
        a1 = jnp.sum(acc[4:8], axis=0, keepdims=True)
        cw2.wait()
        mlp = jnp.dot(act, w2b[...], preferred_element_type=jnp.float32)
        row2 = lax.broadcasted_iota(jnp.int32, (2, D), 0)
        res = xx + jnp.where(row2 == 0, jnp.broadcast_to(a0 + mlp[0:1], (2, D)), jnp.broadcast_to(a1 + mlp[4:5], (2, D)))
        o_ref[...] = res.astype(o_ref.dtype)
    return kernel

@jax.jit
def pallas_parallel_sum__sliding_block_cached__dense_activation_mish__decode_kernel(A_x, A_k_cache, A_v_cache, A_wq, A_wo, B_x, B_w1, B_b1, B_w2):
    SK = A_k_cache.shape[2]
    W = min(4096, max(256, SK // 4))
    bf = jnp.bfloat16
    out = pl.pallas_call(
        make_kernel(W, SK),
        out_shape=jax.ShapeDtypeStruct((B, D), A_x.dtype),
        in_specs=[pl.BlockSpec(memory_space=pl.ANY)] * 8,
        out_specs=pl.BlockSpec(memory_space=pltpu.VMEM),
        scratch_shapes=[
            pltpu.VMEM((B, D), bf),
            pltpu.VMEM((F,), bf),
            pltpu.VMEM((HKV, B, W, DH), bf),
            pltpu.VMEM((HKV, B, W, DH), bf),
            pltpu.VMEM((D, HQ * DH), bf),
            pltpu.VMEM((HKV, 512, D), bf),
            pltpu.VMEM((D, F), bf),
            pltpu.VMEM((F, D), bf),
            pltpu.VMEM((HKV, 8, DH), jnp.float32),
            pltpu.SemaphoreType.DMA((5,)),
        ],
        compiler_params=pltpu.CompilerParams(vmem_limit_bytes=100 * 1024 * 1024),
    )(A_x.reshape(B, D), A_k_cache, A_v_cache, A_wq, A_wo, B_w1, B_b1, B_w2)
    return out.reshape(A_x.shape)
```

```python
import jax, jax.numpy as jnp
from jax import lax
from jax.experimental import pallas as pl
from jax.experimental.pallas import tpu as pltpu

B, D = 2, 512
HQ, HKV, DH = 32, 8, 128
REP = HQ // HKV
F = 1792
NT = (((1,), (1,)), ((), ()))
SP = 6
SPA = 12
CK = 128

S_X, S_WQ, S_W1 = 0, 1, 2
S_K, S_V, S_WO = 3, 5, 7
S_W2 = 9
NSEM = 12

def make_kernel(W, SK):
    NC = W // CK
    HC = NC // 2
    def kernel(x_hbm, k_hbm, v_hbm, wq_hbm, wo_hbm, w1_hbm, b1_hbm, w2_hbm, o_ref,
               xbuf, b1buf, kbuf, vbuf, wqb, wob, w1b, w2b, qscr, pscr, lscr, sems):
        def mo(x, k):
            return x if isinstance(x, int) else pl.multiple_of(x, k)
        def kv_chunk(src, dst, h, b, c, sem, prio):
            off = mo(c * CK, CK)
            pltpu.make_async_copy(src.at[b, h, pl.ds(SK - W + off, CK)], dst.at[h, b, pl.ds(off, CK)], sems.at[sem]).start(priority=prio)
        def wq_chunk(c, prio):
            r = mo((c // 2) * 8, 8); col = mo((c % 2) * 2048, 128)
            pltpu.make_async_copy(wq_hbm.at[pl.ds(r, 8), pl.ds(col, 2048)], wqb.at[pl.ds(r, 8), pl.ds(col, 2048)], sems.at[S_WQ]).start(priority=prio)
        def w1_chunk(c, prio):
            r = mo(c * 8, 8)
            pltpu.make_async_copy(w1_hbm.at[pl.ds(r, 8)], w1b.at[pl.ds(r, 8)], sems.at[S_W1]).start(priority=prio)
        def wo_chunk(h, c, sem, prio):
            r = mo(c * 32, 32)
            pltpu.make_async_copy(wo_hbm.at[pl.ds(mo(h * 512 + r, 32), 32)], wob.at[h, pl.ds(r, 32)], sems.at[sem]).start(priority=prio)
        def w2_chunk(c, sem, prio):
            r = mo(c * 32, 32)
            pltpu.make_async_copy(w2_hbm.at[pl.ds(r, 32)], w2b.at[pl.ds(r, 32)], sems.at[sem]).start(priority=prio)
        def wait_buf(ref, sem):
            pltpu.make_async_copy(ref, ref, sems.at[sem]).wait()

        def loop(lo, hi, body):
            def f(i, c):
                body(i)
                return c
            lax.fori_loop(lo, hi, f, 0)

        def a1(i):
            for j in range(8):
                wq_chunk(j * 16 + i, j % 2)
        a1(0)
        cx = pltpu.make_async_copy(x_hbm, xbuf, sems.at[S_X])
        cb1 = pltpu.make_async_copy(b1_hbm, b1buf, sems.at[S_X])
        cx.start(); cb1.start()
        loop(1, 16, a1)
        def a2(i):
            for s in range(2):
                for b in range(2):
                    kv_chunk(k_hbm, kbuf, 0, b, s * HC + i, S_K, 0)
                    w1_chunk((2 * s + b) * 16 + i, 1)
        loop(0, SPA, a2)

        def ph(g, i2):
            par = g % 2
            n = 0
            for u in range(2):
                i = i2 * 2 + u
                for s in range(2):
                    for b in range(2):
                        kv_chunk(k_hbm, kbuf, g + 1, b, s * HC + i, S_K + 1 - par, n % 2); n += 1
                        kv_chunk(v_hbm, vbuf, g, b, s * HC + i, S_V + par, n % 2); n += 1
                wo_chunk(g, i, S_WO + par, n % 2); n += 1
        def ph7(i2):
            g = HKV - 1
            par = g % 2
            n = 0
            for u in range(2):
                i = i2 * 2 + u
                for s in range(2):
                    for b in range(2):
                        kv_chunk(v_hbm, vbuf, g, b, s * HC + i, S_V + par, n % 2); n += 1
                wo_chunk(g, i, S_WO + par, n % 2); n += 1

        cx.wait(); cb1.wait()
        row = lax.broadcasted_iota(jnp.int32, (8, D), 0)
        xx = xbuf[...].astype(jnp.float32)
        mu = jnp.mean(xx, axis=-1, keepdims=True)
        xc = xx - mu
        var = jnp.mean(xc * xc, axis=-1, keepdims=True)
        xn = xc / jnp.sqrt(var + 1e-5)
        xn0 = jnp.broadcast_to(xn[0:1], (8, D)); xn1 = jnp.broadcast_to(xn[1:2], (8, D))
        xn8b = jnp.where(row < 4, xn0, xn1).astype(jnp.bfloat16)
        xn2b = jnp.where(row % 2 == 0, xn0, xn1).astype(jnp.bfloat16)
        row128 = lax.broadcasted_iota(jnp.int32, (8, DH), 0)
        rowW = lax.broadcasted_iota(jnp.int32, (8, W), 0)
        scale = DH ** -0.5
        wait_buf(wqb, S_WQ)
        qall = jnp.dot(xn8b, wqb[...], preferred_element_type=jnp.float32)
        for h in range(HKV):
            q = qall[:, (4 * h) * 128:(4 * h + 1) * 128]
            for j in range(1, REP):
                q = jnp.where(row128 % 4 == j, qall[:, (4 * h + j) * 128:(4 * h + j + 1) * 128], q)
            qscr[h] = q

        loop(SPA, 16, a2)
        loop(0, SP, lambda i: ph(0, i))

        def qk(h):
            qb = qscr[h].astype(jnp.bfloat16)
            s0 = lax.dot_general(qb, kbuf[h, 0], NT, preferred_element_type=jnp.float32)
            s1 = lax.dot_general(qb, kbuf[h, 1], NT, preferred_element_type=jnp.float32)
            s = jnp.where(rowW < 4, s0, s1) * scale
            m = jnp.max(s, axis=-1, keepdims=True)
            p = jnp.exp(s - m)
            l = jnp.sum(p, axis=-1, keepdims=True)
            pscr[...] = p.astype(jnp.bfloat16)
            lscr[...] = jnp.broadcast_to(l, (8, DH))
        def pv(h, acc):
            pb = pscr[...]
            o0 = jnp.dot(pb, vbuf[h, 0], preferred_element_type=jnp.float32)
            o1 = jnp.dot(pb, vbuf[h, 1], preferred_element_type=jnp.float32)
            o = jnp.where(row128 < 4, o0, o1) / lscr[...]
            for j in range(REP):
                oj = jnp.where(row128 % 4 == j, o, 0.0).astype(jnp.bfloat16)
                acc = acc + jnp.dot(oj, wob[h, j * 128:(j + 1) * 128, :], preferred_element_type=jnp.float32)
            return acc

        wait_buf(kbuf.at[0], S_K)
        qk(0)
        wait_buf(w1b, S_W1)
        hh = jnp.dot(xn2b, w1b[...], preferred_element_type=jnp.float32) + b1buf[...].astype(jnp.float32)[None, :]
        sp = jnp.log1p(jnp.exp(-jnp.abs(hh))) + jnp.maximum(hh, 0.0)
        act = (hh * jnp.tanh(sp)).astype(jnp.bfloat16)

        def step(g, acc, nxt, nsp=SP):
            par = g % 2
            loop(SP, 8, lambda i: ph(g, i))
            loop(0, nsp, nxt)
            wait_buf(vbuf.at[g], S_V + par)
            wait_buf(wob.at[g], S_WO + par)
            wait_buf(kbuf.at[g + 1], S_K + 1 - par)
            acc = pv(g, acc)
            qk(g + 1)
            return acc

        acc = jnp.zeros((8, D), jnp.float32)
        acc = lax.fori_loop(0, HKV - 2, lambda g, acc: step(g, acc, lambda i: ph(g + 1, i)), acc)
        acc = step(HKV - 2, acc, ph7, 8)
        W2G = [(0, 20), (20, 24), (24, 28)]
        for gi, (lo, hi) in enumerate(W2G):
            def w2b_(i, gi=gi):
                w2_chunk(i, S_W2 + gi, 0)
                w2_chunk(28 + i, S_W2 + gi, 1)
            loop(lo, hi, w2b_)
        g = HKV - 1
        wait_buf(vbuf.at[g], S_V + g % 2)
        wait_buf(wob.at[g], S_WO + g % 2)
        acc = pv(g, acc)
        a0 = jnp.sum(acc[0:4], axis=0, keepdims=True)
        a1_ = jnp.sum(acc[4:8], axis=0, keepdims=True)
        row2 = lax.broadcasted_iota(jnp.int32, (2, D), 0)
        res = xx + jnp.where(row2 == 0, jnp.broadcast_to(a0, (2, D)), jnp.broadcast_to(a1_, (2, D)))
        for gi, (lo, hi) in enumerate(W2G):
            rs = [(lo * 32, hi * 32), (896 + lo * 32, 896 + hi * 32)]
            for (a, b) in rs:
                wait_buf(w2b.at[pl.ds(a, b - a)], S_W2 + gi)
            mlp = None
            for (a, b) in rs:
                t = jnp.dot(act[:, a:b], w2b[a:b, :], preferred_element_type=jnp.float32)
                mlp = t if mlp is None else mlp + t
            res = res + mlp[0:2]
        o_ref[...] = res.astype(o_ref.dtype)
    return kernel

@jax.jit
def pallas_parallel_sum__sliding_block_cached__dense_activation_mish__decode_kernel(A_x, A_k_cache, A_v_cache, A_wq, A_wo, B_x, B_w1, B_b1, B_w2):
    SK = A_k_cache.shape[2]
    W = min(4096, max(256, SK // 4))
    bf = jnp.bfloat16
    out = pl.pallas_call(
        make_kernel(W, SK),
        out_shape=jax.ShapeDtypeStruct((B, D), A_x.dtype),
        in_specs=[pl.BlockSpec(memory_space=pl.ANY)] * 8,
        out_specs=pl.BlockSpec(memory_space=pltpu.VMEM),
        scratch_shapes=[
            pltpu.VMEM((B, D), bf),
            pltpu.VMEM((F,), bf),
            pltpu.VMEM((HKV, B, W, DH), bf),
            pltpu.VMEM((HKV, B, W, DH), bf),
            pltpu.VMEM((D, HQ * DH), bf),
            pltpu.VMEM((HKV, 512, D), bf),
            pltpu.VMEM((D, F), bf),
            pltpu.VMEM((F, D), bf),
            pltpu.VMEM((HKV, 8, DH), jnp.float32),
            pltpu.VMEM((8, W), bf),
            pltpu.VMEM((8, DH), jnp.float32),
            pltpu.SemaphoreType.DMA((NSEM,)),
        ],
        compiler_params=pltpu.CompilerParams(vmem_limit_bytes=100 * 1024 * 1024, disable_semaphore_checks=True, disable_bounds_checks=True),
    )(A_x.reshape(B, D), A_k_cache, A_v_cache, A_wq, A_wo, B_w1, B_b1, B_w2)
    return out.reshape(A_x.shape)
```

```python
import functools
import jax, jax.numpy as jnp
from jax import lax
from jax.experimental import pallas as pl
from jax.experimental.pallas import tpu as pltpu

B, D = 2, 512
HQ, HKV, DH = 32, 8, 128
REP = HQ // HKV
F = 1792
NT = (((1,), (1,)), ((), ()))
K = lambda b, h: ("k", b, h)
V = lambda b, h: ("v", b, h)
def aname(a): return a[0] if isinstance(a, tuple) else a
def zipl(*ls):
    out = []
    for i in range(max(len(l) for l in ls)):
        for l in ls:
            if i < len(l): out.append(l[i])
    return out
CB = 32
CK, CW, CQ = 128, 32, 2048
N, H = 32, 16

def plan_stag():
    hw = lambda T, h, s: [(T(b, h), s * H) for b in range(2)]
    wq = lambda half: [("wq", j * N + half * H) for j in range(4)]
    w1 = [("w1", j * H) for j in range(4)]
    wo = lambda h: [("wo", h * H)]
    slots = []
    slots.append(zipl(wq(0), w1))
    slots.append(zipl(wq(1), hw(K, 0, 0) + hw(V, 0, 0)))
    slots.append(zipl(hw(K, 0, 1) + hw(K, 1, 0), wo(0) + wo(2) + wo(4) + wo(6)))
    for g in range(6):
        slots.append(zipl(hw(K, g + 2, 0) + hw(K, g + 1, 1), hw(V, g + 1, 0) + hw(V, g, 1)))
    slots.append(zipl(hw(K, 7, 1) + wo(1) + wo(3), hw(V, 7, 0) + hw(V, 6, 1)))
    slots.append(zipl(hw(V, 7, 1), wo(5) + wo(7)))
    return slots

def build(PAT=(0, 1, 1, 1), GROUPS=(512, 640, 256, 128), VG=(64, 64, 32, 32, 32, 32), NOCOMP=0, LAG=108, N0=None, PH=16):
    NMX = len(GROUPS)
    VROWS = sum(VG)
    GROUPS = tuple(GROUPS) + tuple(VG)
    NP = len(PAT)
    assert sum(GROUPS) == F
    assert 0 <= PH < CK and PH % 8 == 0
    slots = plan_stag()
    seen = set()
    for st in slots:
        for arr, c0 in st:
            for i in range(H):
                assert (arr, c0 + i) not in seen
                seen.add((arr, c0 + i))
    want = {(T(b, h), c) for T in (K, V) for b in range(2) for h in range(8) for c in range(N)}
    want |= {("wq", c) for c in range(128)} | {("wo", c) for c in range(128)} | {("w1", c) for c in range(64)}
    assert seen == want
    NS = len(slots)
    S_X, S_SLOT = 0, 1
    S_W2 = S_SLOT + NS
    NSEM = S_W2 + len(GROUPS)
    def make_kernel(W, SK):
        assert W == N * CK
        def kvb(c):
            return 0 if c == 0 else (W if c == N else c * CK - PH)
        def kernel(x_hbm, k_hbm, v_hbm, wq_hbm, wo_hbm, w1_hbm, b1_hbm, w2_hbm, o_ref,
                   xbuf, b1buf, kbuf, vbuf, wqb, wob, w1b, w2b, qscr, pscr, lscr, oscr, atscr, sems):
            src = dict(k=k_hbm, v=v_hbm, wq=wq_hbm, wo=wo_hbm, w1=w1_hbm, w2=w2_hbm)
            dst = dict(k=kbuf, v=vbuf, wq=wqb, wo=wob, w1=w1b, w2=w2b)
            def mo(x, k):
                return x if isinstance(x, int) else pl.multiple_of(x, k)
            def chunk(arr, c, sem):
                n = aname(arr)
                if n in ("k", "v"):
                    _, b, h = arr
                    if isinstance(c, int):
                        off, sz = kvb(c), kvb(c + 1) - kvb(c)
                    else:
                        off, sz = pl.multiple_of(c * CK - PH, 8), CK
                    s, d = src[n].at[b, h, pl.ds(SK - W + off, sz)], dst[n].at[h, b, pl.ds(off, sz)]
                elif n == "wq":
                    r = mo((c // 2) * 8, 8); col = mo((c % 2) * CQ, 128)
                    s, d = src[n].at[pl.ds(r, 8), pl.ds(col, CQ)], dst[n].at[pl.ds(r, 8), pl.ds(col, CQ)]
                elif n == "w1":
                    r = mo(c * 8, 8)
                    s, d = src[n].at[pl.ds(r, 8)], dst[n].at[pl.ds(r, 8)]
                else:
                    r = mo(c * CW, CW)
                    s, d = src[n].at[pl.ds(r, CW)], dst[n].at[pl.ds(r, CW)]
                return pltpu.make_async_copy(s, d, sems.at[sem])
            def region(arr, c0, n):
                nm = aname(arr)
                if nm in ("k", "v"):
                    _, b, h = arr
                    return dst[nm].at[h, b, pl.ds(kvb(c0), kvb(c0 + n) - kvb(c0))]
                if nm == "wq":
                    return dst[nm].at[pl.ds(c0 // 2 * 8, n // 2 * 8)]
                if nm == "w1":
                    return dst[nm].at[pl.ds(c0 * 8, n * 8)]
                return dst[nm].at[pl.ds(c0 * CW, n * CW)]
            def wait_ref(ref, sem):
                pltpu.make_async_copy(ref, ref, sems.at[sem]).wait()
            def issue(t, lo, hi):
                st = slots[t]
                assert len(st) % NP == 0
                def rnd(i):
                    for n, (arr, c0) in enumerate(st):
                        chunk(arr, c0 + i, S_SLOT + t).start(priority=PAT[n % NP])
                if lo == 0 and hi > 0:
                    rnd(0); lo = 1
                last = hi == H and hi > lo
                if last: hi = H - 1
                if hi > lo:
                    def f(i, c):
                        rnd(i)
                        return c
                    lax.fori_loop(lo, hi, f, 0)
                if last: rnd(H - 1)
            def wait_slot(t):
                for arr, c0 in slots[t]:
                    wait_ref(region(arr, c0, H), S_SLOT + t)

            row = lax.broadcasted_iota(jnp.int32, (8, D), 0)
            row128 = lax.broadcasted_iota(jnp.int32, (8, DH), 0)
            rowW = lax.broadcasted_iota(jnp.int32, (8, W), 0)
            scale = DH ** -0.5
            S = {}
            nbv = -(-VROWS // 128)

            def t_ln():
                xx = xbuf[...].astype(jnp.float32)
                mu = jnp.mean(xx, axis=-1, keepdims=True)
                xc = xx - mu
                var = jnp.mean(xc * xc, axis=-1, keepdims=True)
                xn = xc / jnp.sqrt(var + 1e-5)
                xn0 = jnp.broadcast_to(xn[0:1], (8, D)); xn1 = jnp.broadcast_to(xn[1:2], (8, D))
                S["xx"] = xx
                S["xn8b"] = jnp.where(row < 4, xn0, xn1).astype(jnp.bfloat16)
                S["xn2b"] = jnp.where(row % 2 == 0, xn0, xn1).astype(jnp.bfloat16)
                S["acc"] = jnp.zeros((8, D), jnp.float32)
            def t_mlp1():
                hh = (jnp.zeros((8, F), jnp.float32) if NOCOMP & 4 else jnp.dot(S["xn2b"], w1b[...], preferred_element_type=jnp.float32)) + b1buf[...].astype(jnp.float32)[None, :]
                sp = jnp.log1p(jnp.exp(-jnp.abs(hh))) + jnp.maximum(hh, 0.0)
                S["act"] = (hh * jnp.tanh(sp)).astype(jnp.bfloat16)
                for i in range(nbv):
                    c0 = F - (nbv - i) * 128
                    blk = S["act"][:, c0:c0 + 128].astype(jnp.float32)
                    for b in range(2):
                        atscr[b, i * 128:(i + 1) * 128, :] = jnp.broadcast_to(blk[b:b + 1], (128, 128)).T
            def t_q(h0, h1):
                if NOCOMP & 4: return
                qall = jnp.dot(S["xn8b"], wqb[:, h0 * 512:h1 * 512], preferred_element_type=jnp.float32)
                for h in range(h1 - h0):
                    q = qall[:, (4 * h) * 128:(4 * h + 1) * 128]
                    for j in range(1, REP):
                        q = jnp.where(row128 % 4 == j, qall[:, (4 * h + j) * 128:(4 * h + j + 1) * 128], q)
                    qscr[h0 + h] = q
            def t_qk(h):
                if NOCOMP & 1:
                    pscr[...] = jnp.zeros(pscr.shape, pscr.dtype); lscr[...] = jnp.ones(lscr.shape, lscr.dtype)
                    return
                qb = qscr[h].astype(jnp.bfloat16)
                s0 = lax.dot_general(qb, kbuf[h, 0], NT, preferred_element_type=jnp.float32)
                s1 = lax.dot_general(qb, kbuf[h, 1], NT, preferred_element_type=jnp.float32)
                s = jnp.where(rowW < 4, s0, s1) * scale
                m = jnp.max(s, axis=-1, keepdims=True)
                p = jnp.exp(s - m)
                l = jnp.sum(p, axis=-1, keepdims=True)
                pscr[...] = p.astype(jnp.bfloat16)
                lscr[...] = jnp.broadcast_to(l, (8, DH))
            def t_pv(h):
                if NOCOMP & 2:
                    oscr[h] = jnp.zeros((8, DH), jnp.float32)
                    return
                pb = pscr[...]
                o0 = jnp.dot(pb, vbuf[h, 0], preferred_element_type=jnp.float32)
                o1 = jnp.dot(pb, vbuf[h, 1], preferred_element_type=jnp.float32)
                oscr[h] = jnp.where(row128 < 4, o0, o1) / lscr[...]
            def t_op(h):
                if NOCOMP & 2: return
                o = oscr[h]
                acc = S["acc"]
                for j in range(REP):
                    oj = jnp.where(row128 % 4 == j, o, 0.0).astype(jnp.bfloat16)
                    r0 = h * 512 + j * 128
                    acc = acc + jnp.dot(oj, wob[r0:r0 + 128, :], preferred_element_type=jnp.float32)
                S["acc"] = acc

            after = {
                0: [[t_ln, t_mlp1]],
                1: [[lambda: t_q(0, 4)], [lambda: t_q(4, 8)]],
                2: [[lambda: t_qk(0)]],
            }
            for g in range(7):
                pc = [functools.partial(t_pv, g)]
                if g % 2 == 0: pc.append(functools.partial(t_op, g))
                after[3 + g] = [pc, [functools.partial(t_qk, g + 1)]]
            after[9][1] += [functools.partial(t_op, 1), functools.partial(t_op, 3)]

            issue(0, 0, 1)
            cx = pltpu.make_async_copy(x_hbm, xbuf, sems.at[S_X])
            cb1 = pltpu.make_async_copy(b1_hbm, b1buf, sems.at[S_X])
            cx.start(); cb1.start()
            issue(0, 1, H)
            n2 = F // CW
            goff = [sum(GROUPS[:i]) // CW for i in range(len(GROUPS) + 1)]
            grp_of = lambda c: max(i for i in range(len(GROUPS)) if goff[i] <= c)
            pos0 = [p for p in range(n2) if PAT[p % NP] == 0]
            if N0 is not None: pos0 = pos0[:N0]
            e0 = goff[2]
            L0 = list(range(e0 - len(pos0), e0))
            L1 = [c for c in range(n2) if c not in L0]
            seq = [(L0.pop(0), 0) if p in pos0 else (L1.pop(0), 1) for p in range(n2)]
            assert sorted(c for c, _ in seq) == list(range(n2))
            def issue_w2(lo, hi):
                for c, pr in seq[lo:hi]:
                    chunk("w2", c, S_W2 + grp_of(c)).start(priority=pr)

            for t in range(1, NS):
                per = len(slots[t])
                pieces = after[t - 1]
                r1 = min(H, -(-LAG // per))
                issue(t, 0, r1)
                last = t == NS - 1
                if t == 1:
                    cx.wait(); cb1.wait()
                wait_slot(t - 1)
                r = r1
                for pi, pc in enumerate(pieces):
                    for task in pc: task()
                    if not last:
                        r2 = H if pi == len(pieces) - 1 else (r + H) // 2
                        issue(t, r, r2); r = r2
                    else:
                        if pi == 0:
                            issue(t, r, H); issue_w2(0, n2 // 2)
                        else:
                            issue_w2(n2 // 2, n2)
            wait_slot(NS - 1)
            t_pv(7); t_op(5); t_op(7)
            acc, xx, act = S["acc"], S["xx"], S["act"]
            a0 = jnp.sum(acc[0:4], axis=0, keepdims=True) + xx[0:1]
            a1_ = jnp.sum(acc[4:8], axis=0, keepdims=True) + xx[1:2]
            res = jnp.where(row % 2 == 0, jnp.broadcast_to(a0, (8, D)), jnp.broadcast_to(a1_, (8, D)))
            for gi in range(NMX):
                a, b = goff[gi] * CW, goff[gi + 1] * CW
                wait_ref(w2b.at[pl.ds(a, b - a)], S_W2 + gi)
                if NOCOMP & 8:
                    continue
                res = res + jnp.dot(act[:, a:b], w2b[a:b, :], preferred_element_type=jnp.float32)
            if VROWS:
                base = F - nbv * 128
                acc0 = jnp.where(row == 0, res, 0.0)
                acc1 = jnp.where(row == 1, res, 0.0)
                for gi in range(NMX, len(GROUPS)):
                    a, b = goff[gi] * CW, goff[gi + 1] * CW
                    wait_ref(w2b.at[pl.ds(a, b - a)], S_W2 + gi)
                    if NOCOMP & 8:
                        continue
                    for r in range(a, b, 8):
                        wrow = w2b[r:r + 8, :].astype(jnp.float32)
                        a0v = atscr[0, r - base:r - base + 8, :]
                        a1v = atscr[1, r - base:r - base + 8, :]
                        acc0 = acc0 + wrow * jnp.concatenate([a0v] * 4, axis=1)
                        acc1 = acc1 + wrow * jnp.concatenate([a1v] * 4, axis=1)
                t = jnp.where(row % 2 == 0, acc0 + pltpu.roll(acc0, 7, 0), acc1 + pltpu.roll(acc1, 1, 0))
                t = t + pltpu.roll(t, 2, 0)
                res = t + pltpu.roll(t, 4, 0)
            o_ref[...] = res.astype(o_ref.dtype)[0:2]
        return kernel

    @jax.jit
    def kernel_fn(A_x, A_k_cache, A_v_cache, A_wq, A_wo, B_x, B_w1, B_b1, B_w2):
        SK = A_k_cache.shape[2]
        W = min(4096, max(256, SK // 4))
        bf = jnp.bfloat16
        out = pl.pallas_call(
            make_kernel(W, SK),
            out_shape=jax.ShapeDtypeStruct((B, D), A_x.dtype),
            in_specs=[pl.BlockSpec(memory_space=pl.ANY)] * 8,
            out_specs=pl.BlockSpec(memory_space=pltpu.VMEM),
            scratch_shapes=[
                pltpu.VMEM((B, D), bf),
                pltpu.VMEM((F,), bf),
                pltpu.VMEM((HKV, B, W, DH), bf),
                pltpu.VMEM((HKV, B, W, DH), bf),
                pltpu.VMEM((D, HQ * DH), bf),
                pltpu.VMEM((HQ * DH, D), bf),
                pltpu.VMEM((D, F), bf),
                pltpu.VMEM((F, D), bf),
                pltpu.VMEM((HKV, 8, DH), jnp.float32),
                pltpu.VMEM((8, W), bf),
                pltpu.VMEM((8, DH), jnp.float32),
                pltpu.VMEM((HKV, 8, DH), jnp.float32),
                pltpu.VMEM((2, 256, 128), jnp.float32),
                pltpu.SemaphoreType.DMA((NSEM,)),
            ],
            compiler_params=pltpu.CompilerParams(vmem_limit_bytes=100 * 1024 * 1024, disable_semaphore_checks=True, disable_bounds_checks=True),
        )(A_x.reshape(B, D), A_k_cache, A_v_cache, A_wq, A_wo, B_w1, B_b1, B_w2)
        return out.reshape(A_x.shape)
    return kernel_fn


_KERNEL = build(**dict(PH=16))


def pallas_parallel_sum__sliding_block_cached__dense_activation_mish__decode_kernel(
    A_x, A_k_cache, A_v_cache, A_wq, A_wo, B_x, B_w1, B_b1, B_w2):
    return _KERNEL(A_x, A_k_cache, A_v_cache, A_wq, A_wo, B_x, B_w1, B_b1, B_w2)
```

```python
import functools
import jax, jax.numpy as jnp
from jax import lax
from jax.experimental import pallas as pl
from jax.experimental.pallas import tpu as pltpu

B, D = 2, 512
HQ, HKV, DH = 32, 8, 128
REP = HQ // HKV
F = 1792
NT = (((1,), (1,)), ((), ()))
TPR = dict(k=1, v=1, wq=32, wo=4, w1=14, w2=4)
NTILE = dict(k=512, v=512, wq=2048, wo=2048, w1=896, w2=896)
R = 8

def rects(nm, a, b):
    t = TPR[nm]
    out = []
    while a < b:
        r, c = divmod(a, t)
        if c == 0 and b - a >= t:
            n = (b - a) // t
            out.append((r * 8, n * 8, 0, t * 128)); a += n * t
        else:
            e = min(b, (r + 1) * t)
            out.append((r * 8, 8, c * 128, (e - a) * 128)); a = e
    return out

def blocks(lo, hi, ph, split):
    first = lo + (ph - lo) % 32
    out = []
    last = hi
    if first != lo:
        last = hi - (32 - (first - lo))
        out.append(((last, hi), (lo, first)))
    for a in range(first, last, 32):
        out.append(((a, a + split), (a + split, a + 32)))
    return out

def merge_ranges(rs):
    rs = sorted(rs)
    m = [list(rs[0])]
    for a, b in rs[1:]:
        if a == m[-1][1]: m[-1][1] = b
        else: m.append([a, b])
    return m

def build(PHS=dict(k=14, v=14, wq=14, wo=14, w1=16, w2=18), NOCOMP=0, LAGR=7, ENDF=0.8, VROWS=256, W2R=(4, 6, 8), PRE=100, BCHK=True, W1D=9):
    SPLIT = dict(k=16, v=16, wq=(32 - PHS["wq"]) % 32 or 16, wo=14 if PHS["wo"] % 4 == 2 else 16, w1=16, w2=14 if PHS["w2"] % 4 == 2 else 16)
    bl = {n: blocks(0, NTILE[n], PHS[n], SPLIT[n]) for n in ("k", "v", "wq", "w1")}
    wo_bl = [blocks(h * 256, (h + 1) * 256, PHS["wo"], SPLIT["wo"]) for h in range(8)]
    def win(nm):
        return [(nm, b, bl[nm][s * R + i]) for i in range(R) for s in range(2) for b in range(2)]
    def wq_list(half):
        return [("wq", None, bl["wq"][(2 * j + half) * R + i]) for i in range(R) for j in range(4)]
    w1_list = [("w1", None, bl["w1"][(i * W1D) % 28]) for i in range(28)] + [None] * 4
    def wo_list(hs):
        return [("wo", None, wo_bl[h][i]) for i in range(R) for h in hs]
    p2 = PHS["w2"]
    vt0 = (F - VROWS) // 2
    full2 = [(a, a + 32) for a in range(p2, 896 - 31, 32)]
    pre = [(0, p2)] + [(a, min(b, vt0)) for a, b in full2 if a < vt0]
    post_b = sorted(set([vt0] + [a for a, _ in full2 if a > vt0] + [a + SPLIT["w2"] for a, _ in full2 if a + SPLIT["w2"] > vt0] + [full2[-1][1], 896]))
    post = list(zip(post_b[:-1], post_b[1:]))
    npre = len(pre)
    per = -(-npre // 3)
    w2_order = [pre[s * per + i] for i in range(per) for s in range(3) if s * per + i < npre]
    w2_round = {pre[s * per + i]: i for i in range(per) for s in range(3) if s * per + i < npre}
    W2R = tuple(r for r in W2R if r < per) + (per,)
    def w2_grp(rng): return min(g for g, e in enumerate(W2R) if w2_round[rng] < e)
    WOR = (3, 5, 7, 8)
    S_X, S_WQ, S_W1, S_K, S_V, S_WOA = 0, 1, 2, 3, 5, 7
    S_WOB = 8
    S_W2 = S_WOB + len(WOR)
    S_VP = S_W2 + len(W2R)
    NSEM = S_VP + len(post)
    L0 = []
    for n, (nm, _, blk) in enumerate(wo_list((4, 5, 6, 7))):
        i = n // 4
        g = min(g for g, e in enumerate(WOR) if i < e)
        L0 += [("wo", blk[0], S_WOB + g), ("wo", blk[1], S_WOB + g)]
    L1 = []
    for rng in w2_order:
        a, b = rng
        if b - a > 18:
            L1 += [("w2", (a, a + SPLIT["w2"]), S_W2 + w2_grp(rng)), ("w2", (a + SPLIT["w2"], b), S_W2 + w2_grp(rng))]
        else:
            L1 += [("w2", rng, S_W2 + w2_grp(rng))]
    L1 += [("w2", rng, S_VP + i) for i, rng in enumerate(post)]
    fin = []
    i0 = i1 = 0
    n1e = ENDF * len(L1)
    while i0 < len(L0) or i1 < len(L1):
        if i0 < len(L0) and (i1 >= len(L1) or i0 / len(L0) <= i1 / n1e):
            fin.append(L0[i0] + (0,)); i0 += 1
        else:
            fin.append(L1[i1] + (1,)); i1 += 1
    assert merge_ranges([r for nm, r, s, p in fin if nm == "w2"]) == [[0, 896]]
    assert merge_ranges([r for nm, r, s, p in fin if nm == "wo"] + [r for _, _, b in wo_list((0, 1, 2, 3)) for r in b]) == [[0, 2048]]
    assert merge_ranges([r for e in w1_list if e for r in e[2]]) == [[0, 896]]
    assert merge_ranges([r for h in range(2) for e in wq_list(h) for r in e[2]]) == [[0, 2048]]
    for b_ in range(2):
        assert merge_ranges([r for e in win("k") if e[1] == b_ for r in e[2]]) == [[0, 512]]
    w2_avail = []
    done = set()
    for g in range(len(W2R)):
        m = merge_ranges([r for r in pre if w2_grp(r) <= g])
        new = [j for j in range((F - VROWS) // 128) if j not in done and any(a <= j * 64 and (j + 1) * 64 <= b for a, b in m)]
        done |= set(new)
        w2_avail.append(new)
    assert len(done) == (F - VROWS) // 128
    nbv = VROWS // 128

    def make_kernel(W, SK):
        assert W == 4096
        def kernel(x_hbm, k_hbm, v_hbm, wq_hbm, wo_hbm, w1_hbm, b1_hbm, w2_hbm, o_ref,
                   xbuf, b1buf, kbuf, vbuf, wqb, wob, w1b, w2b, qscr, pscr, lscr, oscr, atscr, sems):
            src = dict(k=k_hbm, v=v_hbm, wq=wq_hbm, wo=wo_hbm, w1=w1_hbm, w2=w2_hbm)
            dst = dict(k=kbuf, v=vbuf, wq=wqb, wo=wob, w1=w1b, w2=w2b)
            def views(n, bh, r0, nr, c0, nc):
                if n in ("k", "v"):
                    b, h = bh
                    return src[n].at[b, h, pl.ds(SK - W + r0, nr)], dst[n].at[h, b, pl.ds(r0, nr)]
                if nc == src[n].shape[1]:
                    return src[n].at[pl.ds(r0, nr)], dst[n].at[pl.ds(r0, nr)]
                return src[n].at[pl.ds(r0, nr), pl.ds(c0, nc)], dst[n].at[pl.ds(r0, nr), pl.ds(c0, nc)]
            def start(n, bh, rng, sem, prio, dyn=None):
                for (r0, nr, c0, nc) in rects(n, *rng):
                    if dyn is not None:
                        r0 = pl.multiple_of(r0 + dyn * (32 // TPR[n] * 8), 8)
                    s, d = views(n, bh, r0, nr, c0, nc)
                    pltpu.make_async_copy(s, d, sems.at[sem]).start(priority=prio)
            def wait_ref(ref, sem):
                pltpu.make_async_copy(ref, ref, sems.at[sem]).wait()
            def wait_rngs(n, rngs, sem):
                for m in merge_ranges(rngs):
                    for rc in rects(n, *m):
                        wait_ref(views(n, None, *rc)[1], sem)
            def issue(A, Bq, lo, hi, loop=True):
                def rnd(i, dyn=None):
                    for j in range(4):
                        for half in range(2):
                            for prio, (lst, h, sem) in enumerate((A, Bq)):
                                e = lst[i * 4 + j]
                                if e is None: continue
                                start(e[0], (e[1], h), e[2][half], sem, prio, dyn)
                if lo == 0 and hi > 0:
                    rnd(0); lo = 1
                if hi <= lo: return
                if loop and hi - lo > 1:
                    def f(i, c):
                        rnd(lo, i)
                        return c
                    lax.fori_loop(0, hi - lo, f, 0)
                else:
                    for i in range(lo, hi): rnd(i)

            row = lax.broadcasted_iota(jnp.int32, (8, D), 0)
            row128 = lax.broadcasted_iota(jnp.int32, (8, DH), 0)
            rowW = lax.broadcasted_iota(jnp.int32, (8, W), 0)
            scale = DH ** -0.5

            def t_qk(h):
                if NOCOMP & 1:
                    pscr[...] = jnp.zeros(pscr.shape, pscr.dtype); lscr[...] = jnp.ones(lscr.shape, lscr.dtype)
                    return
                qb = qscr[h].astype(jnp.bfloat16)
                s0 = lax.dot_general(qb, kbuf[h, 0], NT, preferred_element_type=jnp.float32)
                s1 = lax.dot_general(qb, kbuf[h, 1], NT, preferred_element_type=jnp.float32)
                s = jnp.where(rowW < 4, s0, s1) * scale
                m = jnp.max(s, axis=-1, keepdims=True)
                p = jnp.exp(s - m)
                l = jnp.sum(p, axis=-1, keepdims=True)
                pscr[...] = p.astype(jnp.bfloat16)
                lscr[...] = jnp.broadcast_to(l, (8, DH))
            def t_pv(h):
                if NOCOMP & 2:
                    oscr[h] = jnp.zeros((8, 512), jnp.float32)
                    return
                pb = pscr[...]
                o0 = jnp.dot(pb, vbuf[h, 0], preferred_element_type=jnp.float32)
                o1 = jnp.dot(pb, vbuf[h, 1], preferred_element_type=jnp.float32)
                o = jnp.where(row128 < 4, o0, o1) / lscr[...]
                for j in range(REP):
                    oscr[h, :, j * 128:(j + 1) * 128] = jnp.where(
                        row128 % 2 == 0, jnp.broadcast_to(o[j:j + 1], (8, DH)), jnp.broadcast_to(o[4 + j:5 + j], (8, DH)))
            def t_op(res, h, j0, j1):
                if NOCOMP & 2: return res
                lhs = oscr[h, :, j0 * 128:j1 * 128].astype(jnp.bfloat16)
                return res + jnp.dot(lhs, wob[h * 512 + j0 * 128:h * 512 + j1 * 128, :], preferred_element_type=jnp.float32)

            KW, VW = win("k"), win("v")
            S0 = ((wq_list(0), None, S_WQ), (w1_list, None, S_W1))
            S1 = ((wq_list(1), None, S_WQ), (KW, 0, S_K))
            SG = lambda g: ((KW, g + 1, S_K + (g + 1) % 2), (VW, g, S_V + g % 2))
            S9 = ((VW, 7, S_V + 1), (wo_list((0, 1, 2, 3)), None, S_WOA))

            issue(*S0, 0, 1)
            cx = pltpu.make_async_copy(x_hbm, xbuf, sems.at[S_X])
            cb1 = pltpu.make_async_copy(b1_hbm, b1buf, sems.at[S_X])
            cx.start(); cb1.start()
            issue(*S0, 1, R, loop=False)
            issue(*S1, 0, LAGR)
            cx.wait(); cb1.wait()
            wait_ref(w1b, S_W1)
            xx = xbuf[...].astype(jnp.float32)
            mu = jnp.mean(xx, axis=-1, keepdims=True)
            xc = xx - mu
            var = jnp.mean(xc * xc, axis=-1, keepdims=True)
            xn = xc / jnp.sqrt(var + 1e-5)
            xn0 = jnp.broadcast_to(xn[0:1], (8, D)); xn1 = jnp.broadcast_to(xn[1:2], (8, D))
            xn8b = jnp.where(row < 4, xn0, xn1).astype(jnp.bfloat16)
            xn2b = jnp.where(row % 2 == 0, xn0, xn1).astype(jnp.bfloat16)
            res = jnp.where(row % 2 == 0, jnp.broadcast_to(xx[0:1], (8, D)), jnp.broadcast_to(xx[1:2], (8, D)))
            hh = (jnp.zeros((8, F), jnp.float32) if NOCOMP & 4 else jnp.dot(xn2b, w1b[...], preferred_element_type=jnp.float32)) + b1buf[...].astype(jnp.float32)[None, :]
            sp = jnp.log1p(jnp.exp(-jnp.abs(hh))) + jnp.maximum(hh, 0.0)
            act = (hh * jnp.tanh(sp)).astype(jnp.bfloat16)
            for i in range(nbv):
                c0 = F - (nbv - i) * 128
                blk = act[:, c0:c0 + 128].astype(jnp.float32)
                for b in range(2):
                    atscr[b, i * 128:(i + 1) * 128, :] = jnp.broadcast_to(blk[b:b + 1], (128, 128)).T
            issue(*S1, LAGR, R)
            issue(*SG(0), 0, LAGR)
            wait_ref(wqb, S_WQ)
            wait_ref(kbuf.at[0], S_K)
            if not NOCOMP & 4:
                qall = jnp.dot(xn8b, wqb[...], preferred_element_type=jnp.float32)
                for h in range(HKV):
                    q = qall[:, (4 * h) * 128:(4 * h + 1) * 128]
                    for j in range(1, REP):
                        q = jnp.where(row128 % 4 == j, qall[:, (4 * h + j) * 128:(4 * h + j + 1) * 128], q)
                    qscr[h] = q
            issue(*SG(0), LAGR, R)
            t_qk(0)

            def step(g, nxt):
                issue(*nxt, 0, LAGR)
                wait_ref(vbuf.at[g], S_V + g % 2)
                wait_ref(kbuf.at[g + 1], S_K + (g + 1) % 2)
                t_pv(g)
                issue(*nxt, LAGR, R)
                t_qk(g + 1)
            def body(g, c):
                step(g, SG(g + 1))
                return c
            lax.fori_loop(0, HKV - 2, body, 0)
            step(HKV - 2, S9)
            def issue_fin(lo, hi):
                for nm, rng, sem, pr in fin[lo:hi]:
                    start(nm, None, rng, sem, pr)
            n_a = PRE * len(fin) // 200
            n_b = (len(fin) + n_a) // 2
            issue_fin(0, n_a)
            wait_ref(vbuf.at[7], S_V + 1)
            t_pv(7)
            issue_fin(n_a, n_b)
            wait_ref(wob.at[pl.ds(0, 2048)], S_WOA)
            for h in range(4):
                res = t_op(res, h, 0, 4)
            issue_fin(n_b, len(fin))
            ev = {}
            for pos, (nm, rng, sem, pr) in enumerate(fin):
                ev[sem] = pos + (12 if pr else 0)
            for sem in sorted((s for s in ev if s < S_VP), key=lambda s: ev[s]):
                nm = "wo" if sem < S_W2 else "w2"
                wait_rngs(nm, [r for n_, r, s, p in fin if s == sem], sem)
                if NOCOMP & 8: continue
                if nm == "wo":
                    j = sem - S_WOB
                    for h in range(4, 8):
                        res = t_op(res, h, j, j + 1)
                else:
                    for a, b in merge_ranges([(j, j + 1) for j in w2_avail[sem - S_W2]]) if w2_avail[sem - S_W2] else []:
                        res = res + jnp.dot(act[:, a * 128:b * 128], w2b[a * 128:b * 128, :], preferred_element_type=jnp.float32)
            base = F - VROWS
            row128 = lax.broadcasted_iota(jnp.int32, (8, DH), 0)
            acc0 = [jnp.where(row128 == 0, res[:, c * 128:(c + 1) * 128], 0.0) for c in range(4)]
            acc1 = [jnp.where(row128 == 1, res[:, c * 128:(c + 1) * 128], 0.0) for c in range(4)]
            for i, rng in enumerate(post):
                wait_rngs("w2", [rng], S_VP + i)
                if NOCOMP & 8: continue
                for t in range(*rng):
                    tr, c = divmod(t, 4)
                    r = tr * 8
                    wt = w2b[r:r + 8, c * 128:(c + 1) * 128].astype(jnp.float32)
                    acc0[c] = acc0[c] + wt * atscr[0, r - base:r - base + 8, :]
                    acc1[c] = acc1[c] + wt * atscr[1, r - base:r - base + 8, :]
            acc0 = jnp.concatenate(acc0, axis=1); acc1 = jnp.concatenate(acc1, axis=1)
            t = jnp.where(row % 2 == 0, acc0 + pltpu.roll(acc0, 7, 0), acc1 + pltpu.roll(acc1, 1, 0))
            t = t + pltpu.roll(t, 2, 0)
            res = t + pltpu.roll(t, 4, 0)
            o_ref[...] = res.astype(o_ref.dtype)[0:2]
        return kernel

    @jax.jit
    def kernel_fn(A_x, A_k_cache, A_v_cache, A_wq, A_wo, B_x, B_w1, B_b1, B_w2):
        SK = A_k_cache.shape[2]
        W = min(4096, max(256, SK // 4))
        bf = jnp.bfloat16
        out = pl.pallas_call(
            make_kernel(W, SK),
            out_shape=jax.ShapeDtypeStruct((B, D), A_x.dtype),
            in_specs=[pl.BlockSpec(memory_space=pl.ANY)] * 8,
            out_specs=pl.BlockSpec(memory_space=pltpu.VMEM),
            scratch_shapes=[
                pltpu.VMEM((B, D), bf),
                pltpu.VMEM((F,), bf),
                pltpu.VMEM((HKV, B, W, DH), bf),
                pltpu.VMEM((HKV, B, W, DH), bf),
                pltpu.VMEM((D, HQ * DH), bf),
                pltpu.VMEM((HQ * DH, D), bf),
                pltpu.VMEM((D, F), bf),
                pltpu.VMEM((F, D), bf),
                pltpu.VMEM((HKV, 8, DH), jnp.float32),
                pltpu.VMEM((8, W), bf),
                pltpu.VMEM((8, DH), jnp.float32),
                pltpu.VMEM((HKV, 8, 512), jnp.float32),
                pltpu.VMEM((2, VROWS, 128), jnp.float32),
                pltpu.SemaphoreType.DMA((NSEM,)),
            ],
            compiler_params=pltpu.CompilerParams(vmem_limit_bytes=100 * 1024 * 1024, disable_semaphore_checks=True, disable_bounds_checks=not BCHK),
        )(A_x.reshape(B, D), A_k_cache, A_v_cache, A_wq, A_wo, B_w1, B_b1, B_w2)
        return out.reshape(A_x.shape)
    return kernel_fn


_KERNEL = build(**dict())


def pallas_parallel_sum__sliding_block_cached__dense_activation_mish__decode_kernel(
    A_x, A_k_cache, A_v_cache, A_wq, A_wo, B_x, B_w1, B_b1, B_w2):
    return _KERNEL(A_x, A_k_cache, A_v_cache, A_wq, A_wo, B_x, B_w1, B_b1, B_w2)
```

```python
import functools

import jax
import jax.numpy as jnp
from jax import lax
import jax.experimental.pallas as pl
import jax.experimental.pallas.tpu as pltpu

B, D = 2, 512
HQ, HKV, DH = 32, 8, 128
REP = HQ // HKV
F = 1792
W = 4096
_NT = (((1,), (1,)), ((), ()))

_TPR = dict(k=1, v=1, wq=32, wo=4, w1=14, w2=4)
_NTILE = dict(k=512, v=512, wq=2048, wo=2048, w1=896, w2=896)
_PHASE = dict(k=14, v=14, wq=14, wo=14, w1=16, w2=18)
_SPLIT = dict(k=16, v=16, wq=18, wo=14, w1=16, w2=14)
_BLK = 32
_R = 8
_LAGR = 7
_VROWS = 384
_ENDF = 0.8
_W2R = (4, 6)
_WOR = (3, 5, 7, 8)


def _rects(nm, a, b):
    t = _TPR[nm]
    out = []
    while a < b:
        r, c = divmod(a, t)
        if c == 0 and b - a >= t:
            n = (b - a) // t
            out.append((r * 8, n * 8, 0, t * 128))
            a += n * t
        else:
            e = min(b, (r + 1) * t)
            out.append((r * 8, 8, c * 128, (e - a) * 128))
            a = e
    return out


def _blocks(nm, lo, hi):
    first = lo + (_PHASE[nm] - lo) % _BLK
    last = hi
    out = []
    if first != lo:
        last = hi - (_BLK - (first - lo))
        out.append(((last, hi), (lo, first)))
    for a in range(first, last, _BLK):
        out.append(((a, a + _SPLIT[nm]), (a + _SPLIT[nm], a + _BLK)))
    return out


def _merge(rs):
    rs = sorted(rs)
    m = [list(rs[0])]
    for a, b in rs[1:]:
        assert a >= m[-1][1], "overlapping ranges"
        if a == m[-1][1]:
            m[-1][1] = b
        else:
            m.append([a, b])
    return m


def _covered(rs, a, b):
    return any(x <= a and b <= y for x, y in _merge(rs))


_S_X, _S_WQ, _S_W1, _S_K, _S_V, _S_WOA, _S_WOB = 0, 1, 2, 3, 5, 7, 8


def _make_plan():
    bl = {n: _blocks(n, 0, _NTILE[n]) for n in ("k", "v", "wq", "w1")}
    wo_bl = [_blocks("wo", h * 256, (h + 1) * 256) for h in range(HKV)]

    def win(nm):
        return [(nm, b, bl[nm][s * _R + i], None)
                for i in range(_R) for s in range(2) for b in range(B)]

    def wq_list(half):
        return [("wq", None, bl["wq"][(2 * j + half) * _R + i], None)
                for i in range(_R) for j in range(4)]

    def wo_list(hs, sem=None):
        return [("wo", None, wo_bl[h][i], sem) for i in range(_R) for h in hs]

    n1 = len(bl["w1"])
    w1_all = [("w1", None, bl["w1"][(i * 9) % n1], None) for i in range(n1)]
    early_wo = wo_list((4, 5, 6, 7), _S_WOB)[:8]
    late_wo = wo_list((4, 5, 6, 7))[8:]

    p2, sp2 = _PHASE["w2"], _SPLIT["w2"]
    vt0 = (F - _VROWS) // 2
    full2 = list(range(p2, _NTILE["w2"] - _BLK + 1, _BLK))
    pre = ([(0, p2)] if p2 else []) + [(a, min(a + _BLK, vt0)) for a in full2 if a < vt0]
    cuts = {vt0, full2[-1] + _BLK, _NTILE["w2"]}
    cuts |= {a for a in full2 if a > vt0} | {a + sp2 for a in full2 if a + sp2 > vt0}
    cuts = sorted(cuts)
    post = list(zip(cuts[:-1], cuts[1:]))
    per = -(-len(pre) // 3)
    order = [(i, pre[s * per + i]) for i in range(per) for s in range(3) if s * per + i < len(pre)]
    w2r = tuple(r for r in _W2R if r < per) + (per,)
    s_w2 = _S_WOB + len(_WOR)
    s_vp = s_w2 + len(w2r)
    nsem = s_vp + len(post)

    l0 = []
    for n, (_, _, blk, _) in enumerate(late_wo):
        g = min(g for g, e in enumerate(_WOR) if 2 + n // 4 < e)
        l0 += [("wo", blk[0], _S_WOB + g), ("wo", blk[1], _S_WOB + g)]
    l1 = []
    for i, (a, b) in order:
        sem = s_w2 + min(g for g, e in enumerate(w2r) if i < e)
        if b - a > 18:
            l1 += [("w2", (a, a + sp2), sem), ("w2", (a + sp2, b), sem)]
        else:
            l1 += [("w2", (a, b), sem)]
    l1 += [("w2", rng, s_vp + i) for i, rng in enumerate(post)]
    fin = []
    i0 = i1 = 0
    while i0 < len(l0) or i1 < len(l1):
        if i0 < len(l0) and (i1 >= len(l1) or i0 / len(l0) <= i1 / (_ENDF * len(l1))):
            fin.append(l0[i0] + (0,))
            i0 += 1
        else:
            fin.append(l1[i1] + (1,))
            i1 += 1

    when = {}
    for pos, (_, _, sem, pr) in enumerate(fin):
        when[sem] = pos + (12 if pr else 0)
    early_rngs = [r for e in early_wo for r in e[2]]
    groups = []
    have = dict(wo=[], w2=[])
    todo = dict(wo=list(range(16, 32)), w2=list(range((F - _VROWS) // 128)))
    for sem in sorted((s for s in when if s < s_vp), key=lambda s: when[s]):
        nm = "wo" if sem < s_w2 else "w2"
        rngs = [r for _, r, s, _ in fin if s == sem] + (early_rngs if sem == _S_WOB else [])
        have[nm] += rngs
        ready = [j for j in todo[nm] if _covered(have[nm], j * 64, (j + 1) * 64)]
        todo[nm] = [j for j in todo[nm] if j not in ready]
        groups.append((nm, sem, rngs, ready))
    assert not todo["wo"] and not todo["w2"]

    assert _merge([r for nm, r, _, _ in fin if nm == "w2"]) == [[0, _NTILE["w2"]]]
    assert _merge([r for nm, r, _, _ in fin if nm == "wo"] + early_rngs) == [[1024, 2048]]
    assert _merge([r for e in wo_list((0, 1, 2, 3)) for r in e[2]]) == [[0, 1024]]
    assert _merge([r for e in w1_all for r in e[2]]) == [[0, _NTILE["w1"]]]
    assert _merge([r for h in range(2) for e in wq_list(h) for r in e[2]]) == [[0, _NTILE["wq"]]]
    for nm in ("k", "v"):
        for b in range(B):
            assert _merge([r for e in win(nm) if e[1] == b for r in e[2]]) == [[0, _NTILE[nm]]]
    s0b = w1_all[4:] + early_wo
    assert len(s0b) == 4 * _R
    return dict(kw=win("k"), vw=win("v"), wq0=wq_list(0), wq1=wq_list(1), w1_pre=w1_all[:4],
                s0b=s0b, woa=wo_list((0, 1, 2, 3)), fin=fin, groups=groups, post=post,
                s_vp=s_vp, nsem=nsem)


_PLAN = _make_plan()


def _kernel(x_hbm, k_hbm, v_hbm, wq_hbm, wo_hbm, w1_hbm, b1_hbm, w2_hbm, o_ref,
            xbuf, b1buf, kbuf, vbuf, wqb, wob, w1b, w2b,
            qscr, pscr, lscr, oscr, atscr, sems, *, sk):
    P = _PLAN
    f32, bf16 = jnp.float32, jnp.bfloat16
    src = dict(k=k_hbm, v=v_hbm, wq=wq_hbm, wo=wo_hbm, w1=w1_hbm, w2=w2_hbm)
    dst = dict(k=kbuf, v=vbuf, wq=wqb, wo=wob, w1=w1b, w2=w2b)

    def views(n, bh, r0, nr, c0, nc):
        if n in ("k", "v"):
            b, h = bh
            return src[n].at[b, h, pl.ds(sk - W + r0, nr)], dst[n].at[h, b, pl.ds(r0, nr)]
        if nc == src[n].shape[1]:
            return src[n].at[pl.ds(r0, nr)], dst[n].at[pl.ds(r0, nr)]
        return (src[n].at[pl.ds(r0, nr), pl.ds(c0, nc)],
                dst[n].at[pl.ds(r0, nr), pl.ds(c0, nc)])

    def start(n, bh, rng, sem, prio, shift=None):
        for (r0, nr, c0, nc) in _rects(n, *rng):
            if shift is not None:
                r0 = pl.multiple_of(r0 + shift * (_BLK // _TPR[n] * 8), 8)
            s, d = views(n, bh, r0, nr, c0, nc)
            pltpu.make_async_copy(s, d, sems.at[sem]).start(priority=prio)

    def wait_ref(ref, sem):
        pltpu.make_async_copy(ref, ref, sems.at[sem]).wait()

    def wait_rngs(n, rngs, sem):
        for m in _merge(rngs):
            for rc in _rects(n, *m):
                wait_ref(views(n, None, *rc)[1], sem)

    def issue(slot, lo, hi, loop=True):
        def rnd(i, shift=None):
            for j in range(4):
                for half in range(2):
                    for prio, (lst, h, sem) in enumerate(slot):
                        n, b, blk, sem2 = lst[i * 4 + j]
                        start(n, (b, h), blk[half], sem if sem2 is None else sem2, prio, shift)
        if lo == 0:
            rnd(0)
            lo = 1
        if loop and hi - lo > 1:
            for lst, _, _ in slot:
                for i in range(lo, hi):
                    for j in range(4):
                        a, b0 = lst[i * 4 + j], lst[lo * 4 + j]
                        assert a[:2] == b0[:2] and _BLK % _TPR[a[0]] == 0
                        assert all(x - y == (i - lo) * _BLK for p, q in zip(a[2], b0[2])
                                   for x, y in zip(p, q))

            def body(i, c):
                rnd(lo, i)
                return c
            lax.fori_loop(0, hi - lo, body, 0)
        else:
            for i in range(lo, hi):
                rnd(i)

    row = lax.broadcasted_iota(jnp.int32, (8, D), 0)
    row128 = lax.broadcasted_iota(jnp.int32, (8, DH), 0)
    roww = lax.broadcasted_iota(jnp.int32, (8, W), 0)

    def scores(h):
        qb = qscr[h].astype(bf16)
        s0 = lax.dot_general(qb, kbuf[h, 0], _NT, preferred_element_type=f32)
        s1 = lax.dot_general(qb, kbuf[h, 1], _NT, preferred_element_type=f32)
        s = jnp.where(roww < REP, s0, s1) * (DH ** -0.5)
        m = jnp.max(s, axis=-1, keepdims=True)
        p = jnp.exp(s - m)
        pscr[...] = p.astype(bf16)
        lscr[...] = jnp.broadcast_to(jnp.sum(p, axis=-1, keepdims=True), (8, DH))

    def values(h):
        pb = pscr[...]
        o0 = jnp.dot(pb, vbuf[h, 0], preferred_element_type=f32)
        o1 = jnp.dot(pb, vbuf[h, 1], preferred_element_type=f32)
        o = jnp.where(row128 < REP, o0, o1) / lscr[...]
        for j in range(REP):
            oscr[h, :, j * DH:(j + 1) * DH] = jnp.where(
                row128 % 2 == 0,
                jnp.broadcast_to(o[j:j + 1], (8, DH)),
                jnp.broadcast_to(o[REP + j:REP + j + 1], (8, DH)))

    def out_proj(res, h, j0, j1):
        lhs = oscr[h, :, j0 * DH:j1 * DH].astype(bf16)
        r0 = h * REP * DH
        return res + jnp.dot(lhs, wob[r0 + j0 * DH:r0 + j1 * DH, :], preferred_element_type=f32)

    slot0 = ((P["wq0"], None, _S_WQ), (P["s0b"], None, _S_W1))
    slot1 = ((P["wq1"], None, _S_WQ), (P["kw"], 0, _S_K))
    slot_kv = lambda g: ((P["kw"], g + 1, _S_K + (g + 1) % 2), (P["vw"], g, _S_V + g % 2))
    slot9 = ((P["vw"], HKV - 1, _S_V + (HKV - 1) % 2), (P["woa"], None, _S_WOA))

    for e in P["w1_pre"]:
        for half in range(2):
            start("w1", None, e[2][half], _S_W1, 1)
    issue(slot0, 0, 1)
    cx = pltpu.make_async_copy(x_hbm, xbuf, sems.at[_S_X])
    cb1 = pltpu.make_async_copy(b1_hbm, b1buf, sems.at[_S_X])
    cx.start()
    cb1.start()
    issue(slot0, 1, _R, loop=False)
    issue(slot1, 0, _LAGR)
    cx.wait()
    cb1.wait()
    wait_ref(w1b, _S_W1)

    xx = xbuf[...].astype(f32)
    mu = jnp.mean(xx, axis=-1, keepdims=True)
    xc = xx - mu
    var = jnp.mean(xc * xc, axis=-1, keepdims=True)
    xn = xc / jnp.sqrt(var + 1e-5)
    xn0 = jnp.broadcast_to(xn[0:1], (8, D))
    xn1 = jnp.broadcast_to(xn[1:2], (8, D))
    xn_q = jnp.where(row < REP, xn0, xn1).astype(bf16)
    xn_m = jnp.where(row % 2 == 0, xn0, xn1).astype(bf16)
    res = jnp.where(row % 2 == 0, jnp.broadcast_to(xx[0:1], (8, D)),
                    jnp.broadcast_to(xx[1:2], (8, D)))

    hh = jnp.dot(xn_m, w1b[...], preferred_element_type=f32) + b1buf[...].astype(f32)[None, :]
    sp = jnp.log1p(jnp.exp(-jnp.abs(hh))) + jnp.maximum(hh, 0.0)
    act = (hh * jnp.tanh(sp)).astype(bf16)
    vbase = F - _VROWS
    for i in range(_VROWS // 128):
        blk = act[:, vbase + i * 128:vbase + (i + 1) * 128].astype(f32)
        for b in range(B):
            atscr[b, i * 128:(i + 1) * 128, :] = jnp.broadcast_to(blk[b:b + 1], (128, 128)).T

    issue(slot1, _LAGR, _R)
    issue(slot_kv(0), 0, _LAGR)
    wait_ref(wqb, _S_WQ)
    wait_ref(kbuf.at[0], _S_K)
    qall = jnp.dot(xn_q, wqb[...], preferred_element_type=f32)
    for h in range(HKV):
        q = qall[:, REP * h * DH:(REP * h + 1) * DH]
        for j in range(1, REP):
            q = jnp.where(row128 % REP == j, qall[:, (REP * h + j) * DH:(REP * h + j + 1) * DH], q)
        qscr[h] = q
    issue(slot_kv(0), _LAGR, _R)
    scores(0)

    def step(g, nxt):
        issue(nxt, 0, _LAGR)
        wait_ref(vbuf.at[g], _S_V + g % 2)
        wait_ref(kbuf.at[g + 1], _S_K + (g + 1) % 2)
        values(g)
        issue(nxt, _LAGR, _R)
        scores(g + 1)

    def loop_body(g, c):
        step(g, slot_kv(g + 1))
        return c
    lax.fori_loop(0, HKV - 2, loop_body, 0)
    step(HKV - 2, slot9)

    fin = P["fin"]

    def issue_fin(lo, hi):
        for nm, rng, sem, pr in fin[lo:hi]:
            start(nm, None, rng, sem, pr)
    n_a = len(fin) // 2
    n_b = (len(fin) + n_a) // 2
    issue_fin(0, n_a)
    wait_ref(vbuf.at[HKV - 1], _S_V + (HKV - 1) % 2)
    values(HKV - 1)
    issue_fin(n_a, n_b)
    wait_ref(wob.at[pl.ds(0, 4 * REP * DH)], _S_WOA)
    for h in range(4):
        res = out_proj(res, h, 0, REP)
    issue_fin(n_b, len(fin))

    for nm, sem, rngs, ready in P["groups"]:
        wait_rngs(nm, rngs, sem)
        if nm == "wo":
            for j in ready:
                res = out_proj(res, j // REP, j % REP, j % REP + 1)
        elif ready:
            for a, b in _merge([(j * 128, (j + 1) * 128) for j in ready]):
                res = res + jnp.dot(act[:, a:b], w2b[a:b, :], preferred_element_type=f32)

    acc0 = [jnp.where(row128 == 0, res[:, c * 128:(c + 1) * 128], 0.0) for c in range(4)]
    acc1 = [jnp.where(row128 == 1, res[:, c * 128:(c + 1) * 128], 0.0) for c in range(4)]
    for i, rng in enumerate(P["post"]):
        wait_rngs("w2", [rng], P["s_vp"] + i)
        for t in range(*rng):
            tr, c = divmod(t, 4)
            r = tr * 8
            wt = w2b[r:r + 8, c * 128:(c + 1) * 128].astype(f32)
            acc0[c] = acc0[c] + wt * atscr[0, r - vbase:r - vbase + 8, :]
            acc1[c] = acc1[c] + wt * atscr[1, r - vbase:r - vbase + 8, :]
    acc0 = jnp.concatenate(acc0, axis=1)
    acc1 = jnp.concatenate(acc1, axis=1)
    t = jnp.where(row % 2 == 0, acc0 + pltpu.roll(acc0, 7, 0), acc1 + pltpu.roll(acc1, 1, 0))
    t = t + pltpu.roll(t, 2, 0)
    t = t + pltpu.roll(t, 4, 0)
    o_ref[...] = t.astype(o_ref.dtype)[0:B]


def _compiler_params():
    kw = dict(vmem_limit_bytes=100 * 1024 * 1024)
    try:
        return pltpu.CompilerParams(disable_semaphore_checks=True, **kw)
    except TypeError:
        return pltpu.CompilerParams(**kw)


@jax.jit
def pallas_parallel_sum__sliding_block_cached__dense_activation_mish__decode_kernel(
    A_x: jax.Array,
    A_k_cache: jax.Array,
    A_v_cache: jax.Array,
    A_wq: jax.Array,
    A_wo: jax.Array,
    B_x: jax.Array,
    B_w1: jax.Array,
    B_b1: jax.Array,
    B_w2: jax.Array,
):
    sk = A_k_cache.shape[2]
    assert A_x.shape == (B, 1, D) and A_k_cache.shape == (B, HKV, sk, DH)
    assert min(4096, max(256, sk // 4)) == W and sk % 8 == 0
    assert A_wq.shape == (D, HQ * DH) and A_wo.shape == (HQ * DH, D)
    assert B_w1.shape == (D, F) and B_w2.shape == (F, D) and B_b1.shape == (F,)
    bf16, f32 = jnp.bfloat16, jnp.float32
    out = pl.pallas_call(
        functools.partial(_kernel, sk=sk),
        out_shape=jax.ShapeDtypeStruct((B, D), A_x.dtype),
        in_specs=[pl.BlockSpec(memory_space=pl.ANY)] * 8,
        out_specs=pl.BlockSpec(memory_space=pltpu.VMEM),
        scratch_shapes=[
            pltpu.VMEM((B, D), bf16),
            pltpu.VMEM((F,), bf16),
            pltpu.VMEM((HKV, B, W, DH), bf16),
            pltpu.VMEM((HKV, B, W, DH), bf16),
            pltpu.VMEM((D, HQ * DH), bf16),
            pltpu.VMEM((HQ * DH, D), bf16),
            pltpu.VMEM((D, F), bf16),
            pltpu.VMEM((F, D), bf16),
            pltpu.VMEM((HKV, 8, DH), f32),
            pltpu.VMEM((8, W), bf16),
            pltpu.VMEM((8, DH), f32),
            pltpu.VMEM((HKV, 8, REP * DH), f32),
            pltpu.VMEM((B, _VROWS, 128), f32),
            pltpu.SemaphoreType.DMA((_PLAN["nsem"],)),
        ],
        compiler_params=_compiler_params(),
    )(A_x.reshape(B, D), A_k_cache, A_v_cache, A_wq, A_wo, B_w1, B_b1, B_w2)
    return out.reshape(A_x.shape)
```

```python
import functools

import jax
import jax.numpy as jnp
from jax import lax
import jax.experimental.pallas as pl
import jax.experimental.pallas.tpu as pltpu

B, D = 2, 512
HQ, HKV, DH = 32, 8, 128
REP = HQ // HKV
F = 1792
W = 4096
_NT = (((1,), (1,)), ((), ()))

_TPR = dict(k=1, v=1, wq=32, wo=4, w1=14, w2=4)
_NTILE = dict(k=512, v=512, wq=2048, wo=2048, w1=896, w2=896)
_PHASE = dict(k=14, v=14, wq=14, wo=14, w1=16, w2=18)
_SPLIT = dict(k=16, v=16, wq=18, wo=14, w1=16, w2=14)
_BLK = 32
_R = 8
_LAGR = 7
_VROWS = 384
_ENDF = 0.8
_W2R = (4, 6)
_WOR = (3, 5, 7, 8)


def _rects(nm, a, b):
    t = _TPR[nm]
    out = []
    while a < b:
        r, c = divmod(a, t)
        if c == 0 and b - a >= t:
            n = (b - a) // t
            out.append((r * 8, n * 8, 0, t * 128))
            a += n * t
        else:
            e = min(b, (r + 1) * t)
            out.append((r * 8, 8, c * 128, (e - a) * 128))
            a = e
    return out


def _blocks(nm, lo, hi):
    first = lo + (_PHASE[nm] - lo) % _BLK
    last = hi
    out = []
    if first != lo:
        last = hi - (_BLK - (first - lo))
        out.append(((last, hi), (lo, first)))
    for a in range(first, last, _BLK):
        out.append(((a, a + _SPLIT[nm]), (a + _SPLIT[nm], a + _BLK)))
    return out


def _merge(rs):
    rs = sorted(rs)
    m = [list(rs[0])]
    for a, b in rs[1:]:
        assert a >= m[-1][1], "overlapping ranges"
        if a == m[-1][1]:
            m[-1][1] = b
        else:
            m.append([a, b])
    return m


def _covered(rs, a, b):
    return any(x <= a and b <= y for x, y in _merge(rs))


_S_X, _S_WQ, _S_W1, _S_K, _S_V, _S_WOA, _S_WOB = 0, 1, 2, 3, 5, 7, 8


def _make_plan():
    bl = {n: _blocks(n, 0, _NTILE[n]) for n in ("k", "v", "wq", "w1")}
    wo_bl = [_blocks("wo", h * 256, (h + 1) * 256) for h in range(HKV)]

    def win(nm):
        return [(nm, b, bl[nm][s * _R + i], None)
                for i in range(_R) for s in range(2) for b in range(B)]

    def wq_list(half):
        return [("wq", None, bl["wq"][(2 * j + half) * _R + i], None)
                for i in range(_R) for j in range(4)]

    def wo_list(hs, sem=None):
        return [("wo", None, wo_bl[h][i], sem) for i in range(_R) for h in hs]

    n1 = len(bl["w1"])
    w1_all = [("w1", None, bl["w1"][(i * 9) % n1], None) for i in range(n1)]
    early_wo = wo_list((4, 5, 6, 7), _S_WOB)[:8]
    late_wo = wo_list((4, 5, 6, 7))[8:]

    p2, sp2 = _PHASE["w2"], _SPLIT["w2"]
    vt0 = (F - _VROWS) // 2
    full2 = list(range(p2, _NTILE["w2"] - _BLK + 1, _BLK))
    pre = ([(0, p2)] if p2 else []) + [(a, min(a + _BLK, vt0)) for a in full2 if a < vt0]
    cuts = {vt0, full2[-1] + _BLK, _NTILE["w2"] - 8, _NTILE["w2"]}
    cuts |= {a for a in full2 if a > vt0} | {a + sp2 for a in full2 if a + sp2 > vt0}
    cuts = sorted(cuts)
    post = list(zip(cuts[:-1], cuts[1:]))
    per = -(-len(pre) // 3)
    order = [(i, pre[s * per + i]) for i in range(per) for s in range(3) if s * per + i < len(pre)]
    w2r = tuple(r for r in _W2R if r < per) + (per,)
    s_w2 = _S_WOB + len(_WOR)
    s_vp = s_w2 + len(w2r)
    nsem = s_vp + len(post)

    l0 = []
    for n, (_, _, blk, _) in enumerate(late_wo):
        g = min(g for g, e in enumerate(_WOR) if 2 + n // 4 < e)
        l0 += [("wo", blk[0], _S_WOB + g), ("wo", blk[1], _S_WOB + g)]
    l1 = []
    for i, (a, b) in order:
        sem = s_w2 + min(g for g, e in enumerate(w2r) if i < e)
        if b - a > 18:
            l1 += [("w2", (a, a + sp2), sem), ("w2", (a + sp2, b), sem)]
        else:
            l1 += [("w2", (a, b), sem)]
    l1 += [("w2", rng, s_vp + i) for i, rng in enumerate(post)]
    fin = []
    i0 = i1 = 0
    while i0 < len(l0) or i1 < len(l1):
        if i0 < len(l0) and (i1 >= len(l1) or i0 / len(l0) <= i1 / (_ENDF * len(l1))):
            fin.append(l0[i0] + (0,))
            i0 += 1
        else:
            fin.append(l1[i1] + (1,))
            i1 += 1

    when = {}
    for pos, (_, _, sem, pr) in enumerate(fin):
        when[sem] = pos + (12 if pr else 0)
    early_rngs = [r for e in early_wo for r in e[2]]
    groups = []
    have = dict(wo=[], w2=[])
    todo = dict(wo=list(range(16, 32)), w2=list(range((F - _VROWS) // 128)))
    for sem in sorted((s for s in when if s < s_vp), key=lambda s: when[s]):
        nm = "wo" if sem < s_w2 else "w2"
        rngs = [r for _, r, s, _ in fin if s == sem] + (early_rngs if sem == _S_WOB else [])
        have[nm] += rngs
        ready = [j for j in todo[nm] if _covered(have[nm], j * 64, (j + 1) * 64)]
        todo[nm] = [j for j in todo[nm] if j not in ready]
        groups.append((nm, sem, rngs, ready))
    assert not todo["wo"] and not todo["w2"]

    assert _merge([r for nm, r, _, _ in fin if nm == "w2"]) == [[0, _NTILE["w2"]]]
    assert _merge([r for nm, r, _, _ in fin if nm == "wo"] + early_rngs) == [[1024, 2048]]
    assert _merge([r for e in wo_list((0, 1, 2, 3)) for r in e[2]]) == [[0, 1024]]
    assert _merge([r for e in w1_all for r in e[2]]) == [[0, _NTILE["w1"]]]
    assert _merge([r for h in range(2) for e in wq_list(h) for r in e[2]]) == [[0, _NTILE["wq"]]]
    for nm in ("k", "v"):
        for b in range(B):
            assert _merge([r for e in win(nm) if e[1] == b for r in e[2]]) == [[0, _NTILE[nm]]]
    s0b = w1_all[4:] + early_wo
    assert len(s0b) == 4 * _R
    return dict(kw=win("k"), vw=win("v"), wq0=wq_list(0), wq1=wq_list(1), w1_pre=w1_all[:4],
                s0b=s0b, woa=wo_list((0, 1, 2, 3)), fin=fin, groups=groups, post=post,
                s_vp=s_vp, nsem=nsem)


_PLAN = _make_plan()


def _kernel(x_hbm, k_hbm, v_hbm, wq_hbm, wo_hbm, w1_hbm, b1_hbm, w2_hbm, o_ref,
            xbuf, b1buf, kbuf, vbuf, wqb, wob, w1b, w2b,
            qscr, pscr, lscr, oscr, atscr, sems, *, sk):
    P = _PLAN
    f32, bf16 = jnp.float32, jnp.bfloat16
    src = dict(k=k_hbm, v=v_hbm, wq=wq_hbm, wo=wo_hbm, w1=w1_hbm, w2=w2_hbm)
    dst = dict(k=kbuf, v=vbuf, wq=wqb, wo=wob, w1=w1b, w2=w2b)

    def views(n, bh, r0, nr, c0, nc):
        if n in ("k", "v"):
            b, h = bh
            return src[n].at[b, h, pl.ds(sk - W + r0, nr)], dst[n].at[h, b, pl.ds(r0, nr)]
        if nc == src[n].shape[1]:
            return src[n].at[pl.ds(r0, nr)], dst[n].at[pl.ds(r0, nr)]
        return (src[n].at[pl.ds(r0, nr), pl.ds(c0, nc)],
                dst[n].at[pl.ds(r0, nr), pl.ds(c0, nc)])

    def start(n, bh, rng, sem, prio, shift=None):
        for (r0, nr, c0, nc) in _rects(n, *rng):
            if shift is not None:
                r0 = pl.multiple_of(r0 + shift * (_BLK // _TPR[n] * 8), 8)
            s, d = views(n, bh, r0, nr, c0, nc)
            pltpu.make_async_copy(s, d, sems.at[sem]).start(priority=prio)

    def wait_ref(ref, sem):
        pltpu.make_async_copy(ref, ref, sems.at[sem]).wait()

    def wait_rngs(n, rngs, sem):
        for rng in rngs:
            for rc in _rects(n, *rng):
                s, d = views(n, None, *rc)
                pltpu.make_async_copy(s, d, sems.at[sem]).wait()

    def issue(slot, lo, hi, loop=True):
        def rnd(i, shift=None):
            for j in range(4):
                for half in range(2):
                    for prio, (lst, h, sem) in enumerate(slot):
                        n, b, blk, sem2 = lst[i * 4 + j]
                        start(n, (b, h), blk[half], sem if sem2 is None else sem2, prio, shift)
        if lo == 0:
            rnd(0)
            lo = 1
        if loop and hi - lo > 1:
            for lst, _, _ in slot:
                for i in range(lo, hi):
                    for j in range(4):
                        a, b0 = lst[i * 4 + j], lst[lo * 4 + j]
                        assert a[:2] == b0[:2] and _BLK % _TPR[a[0]] == 0
                        assert all(x - y == (i - lo) * _BLK for p, q in zip(a[2], b0[2])
                                   for x, y in zip(p, q))

            def body(i, c):
                rnd(lo, i)
                return c
            lax.fori_loop(0, hi - lo, body, 0)
        else:
            for i in range(lo, hi):
                rnd(i)

    row = lax.broadcasted_iota(jnp.int32, (8, D), 0)
    row128 = lax.broadcasted_iota(jnp.int32, (8, DH), 0)
    roww = lax.broadcasted_iota(jnp.int32, (8, W), 0)

    def scores(h):
        qb = qscr[h].astype(bf16)
        s0 = lax.dot_general(qb, kbuf[h, 0], _NT, preferred_element_type=f32)
        s1 = lax.dot_general(qb, kbuf[h, 1], _NT, preferred_element_type=f32)
        s = jnp.where(roww < REP, s0, s1) * (DH ** -0.5)
        m = jnp.max(s, axis=-1, keepdims=True)
        p = jnp.exp(s - m)
        pscr[...] = p.astype(bf16)
        lscr[...] = jnp.broadcast_to(jnp.sum(p, axis=-1, keepdims=True), (8, DH))

    def values(h):
        pb = pscr[...]
        o0 = jnp.dot(pb, vbuf[h, 0], preferred_element_type=f32)
        o1 = jnp.dot(pb, vbuf[h, 1], preferred_element_type=f32)
        o = jnp.where(row128 < REP, o0, o1) / lscr[...]
        for j in range(REP):
            oscr[h, :, j * DH:(j + 1) * DH] = jnp.where(
                row128 % 2 == 0,
                jnp.broadcast_to(o[j:j + 1], (8, DH)),
                jnp.broadcast_to(o[REP + j:REP + j + 1], (8, DH)))

    def out_proj(res, h, j0, j1):
        lhs = oscr[h, :, j0 * DH:j1 * DH].astype(bf16)
        r0 = h * REP * DH
        return res + jnp.dot(lhs, wob[r0 + j0 * DH:r0 + j1 * DH, :], preferred_element_type=f32)

    slot0 = ((P["wq0"], None, _S_WQ), (P["s0b"], None, _S_W1))
    slot1 = ((P["wq1"], None, _S_WQ), (P["kw"], 0, _S_K))
    slot_kv = lambda g: ((P["kw"], g + 1, _S_K + (g + 1) % 2), (P["vw"], g, _S_V + g % 2))
    slot9 = ((P["vw"], HKV - 1, _S_V + (HKV - 1) % 2), (P["woa"], None, _S_WOA))

    for e in P["w1_pre"]:
        for half in range(2):
            start("w1", None, e[2][half], _S_W1, 1)
    issue(slot0, 0, 1)
    cx = pltpu.make_async_copy(x_hbm, xbuf, sems.at[_S_X])
    cb1 = pltpu.make_async_copy(b1_hbm, b1buf, sems.at[_S_X])
    cx.start()
    cb1.start()
    issue(slot0, 1, _R, loop=False)
    issue(slot1, 0, _LAGR)
    cx.wait()
    cb1.wait()
    wait_ref(w1b, _S_W1)

    xx = xbuf[...].astype(f32)
    mu = jnp.mean(xx, axis=-1, keepdims=True)
    xc = xx - mu
    var = jnp.mean(xc * xc, axis=-1, keepdims=True)
    xn = xc / jnp.sqrt(var + 1e-5)
    xn0 = jnp.broadcast_to(xn[0:1], (8, D))
    xn1 = jnp.broadcast_to(xn[1:2], (8, D))
    xn_q = jnp.where(row < REP, xn0, xn1).astype(bf16)
    xn_m = jnp.where(row % 2 == 0, xn0, xn1).astype(bf16)
    res = jnp.where(row % 2 == 0, jnp.broadcast_to(xx[0:1], (8, D)),
                    jnp.broadcast_to(xx[1:2], (8, D)))

    hh = jnp.dot(xn_m, w1b[...], preferred_element_type=f32) + b1buf[...].astype(f32)[None, :]
    sp = jnp.log1p(jnp.exp(-jnp.abs(hh))) + jnp.maximum(hh, 0.0)
    act = (hh * jnp.tanh(sp)).astype(bf16)
    vbase = F - _VROWS
    for i in range(_VROWS // 128):
        blk = act[:, vbase + i * 128:vbase + (i + 1) * 128].astype(f32)
        for b in range(B):
            atscr[b, i * 128:(i + 1) * 128, :] = jnp.broadcast_to(blk[b:b + 1], (128, 128)).T

    issue(slot1, _LAGR, _R)
    issue(slot_kv(0), 0, _LAGR)
    wait_ref(wqb, _S_WQ)
    wait_ref(kbuf.at[0], _S_K)
    qall = jnp.dot(xn_q, wqb[...], preferred_element_type=f32)
    for h in range(HKV):
        q = qall[:, REP * h * DH:(REP * h + 1) * DH]
        for j in range(1, REP):
            q = jnp.where(row128 % REP == j, qall[:, (REP * h + j) * DH:(REP * h + j + 1) * DH], q)
        qscr[h] = q
    issue(slot_kv(0), _LAGR, _R)
    scores(0)

    def step(g, nxt):
        issue(nxt, 0, _LAGR)
        wait_ref(vbuf.at[g], _S_V + g % 2)
        wait_ref(kbuf.at[g + 1], _S_K + (g + 1) % 2)
        values(g)
        issue(nxt, _LAGR, _R)
        scores(g + 1)

    def loop_body(g, c):
        step(g, slot_kv(g + 1))
        return c
    lax.fori_loop(0, HKV - 2, loop_body, 0)
    step(HKV - 2, slot9)

    fin = P["fin"]

    def issue_fin(lo, hi):
        for nm, rng, sem, pr in fin[lo:hi]:
            start(nm, None, rng, sem, pr)
    n_a = len(fin) // 2
    n_b = (len(fin) + n_a) // 2
    issue_fin(0, n_a)
    wait_ref(vbuf.at[HKV - 1], _S_V + (HKV - 1) % 2)
    values(HKV - 1)
    issue_fin(n_a, n_b)
    wait_ref(wob.at[pl.ds(0, 4 * REP * DH)], _S_WOA)
    for h in range(4):
        res = out_proj(res, h, 0, REP)
    issue_fin(n_b, len(fin))

    for nm, sem, rngs, ready in P["groups"]:
        wait_rngs(nm, rngs, sem)
        if nm == "wo":
            for j in ready:
                res = out_proj(res, j // REP, j % REP, j % REP + 1)
        elif ready:
            for a, b in _merge([(j * 128, (j + 1) * 128) for j in ready]):
                res = res + jnp.dot(act[:, a:b], w2b[a:b, :], preferred_element_type=f32)

    acc0 = [jnp.where(row128 == 0, res[:, c * 128:(c + 1) * 128], 0.0) for c in range(4)]
    acc1 = [jnp.where(row128 == 1, res[:, c * 128:(c + 1) * 128], 0.0) for c in range(4)]
    for i, rng in enumerate(P["post"]):
        wait_rngs("w2", [rng], P["s_vp"] + i)
        for t in range(*rng):
            tr, c = divmod(t, 4)
            r = tr * 8
            wt = w2b[r:r + 8, c * 128:(c + 1) * 128].astype(f32)
            acc0[c] = acc0[c] + wt * atscr[0, r - vbase:r - vbase + 8, :]
            acc1[c] = acc1[c] + wt * atscr[1, r - vbase:r - vbase + 8, :]
    acc0 = jnp.concatenate(acc0, axis=1)
    acc1 = jnp.concatenate(acc1, axis=1)
    t = jnp.where(row % 2 == 0, acc0 + pltpu.roll(acc0, 7, 0), acc1 + pltpu.roll(acc1, 1, 0))
    t = t + pltpu.roll(t, 2, 0)
    t = t + pltpu.roll(t, 4, 0)
    o_ref[...] = t.astype(o_ref.dtype)[0:B]


def _compiler_params():
    kw = dict(vmem_limit_bytes=100 * 1024 * 1024)
    try:
        return pltpu.CompilerParams(disable_semaphore_checks=True, **kw)
    except TypeError:
        return pltpu.CompilerParams(**kw)


@jax.jit
def pallas_parallel_sum__sliding_block_cached__dense_activation_mish__decode_kernel(
    A_x: jax.Array,
    A_k_cache: jax.Array,
    A_v_cache: jax.Array,
    A_wq: jax.Array,
    A_wo: jax.Array,
    B_x: jax.Array,
    B_w1: jax.Array,
    B_b1: jax.Array,
    B_w2: jax.Array,
):
    sk = A_k_cache.shape[2]
    assert A_x.shape == (B, 1, D) and A_k_cache.shape == (B, HKV, sk, DH)
    assert min(4096, max(256, sk // 4)) == W and sk % 8 == 0
    assert A_wq.shape == (D, HQ * DH) and A_wo.shape == (HQ * DH, D)
    assert B_w1.shape == (D, F) and B_w2.shape == (F, D) and B_b1.shape == (F,)
    bf16, f32 = jnp.bfloat16, jnp.float32
    out = pl.pallas_call(
        functools.partial(_kernel, sk=sk),
        out_shape=jax.ShapeDtypeStruct((B, D), A_x.dtype),
        in_specs=[pl.BlockSpec(memory_space=pl.ANY)] * 8,
        out_specs=pl.BlockSpec(memory_space=pltpu.VMEM),
        scratch_shapes=[
            pltpu.VMEM((B, D), bf16),
            pltpu.VMEM((F,), bf16),
            pltpu.VMEM((HKV, B, W, DH), bf16),
            pltpu.VMEM((HKV, B, W, DH), bf16),
            pltpu.VMEM((D, HQ * DH), bf16),
            pltpu.VMEM((HQ * DH, D), bf16),
            pltpu.VMEM((D, F), bf16),
            pltpu.VMEM((F, D), bf16),
            pltpu.VMEM((HKV, 8, DH), f32),
            pltpu.VMEM((8, W), bf16),
            pltpu.VMEM((8, DH), f32),
            pltpu.VMEM((HKV, 8, REP * DH), f32),
            pltpu.VMEM((B, _VROWS, 128), f32),
            pltpu.SemaphoreType.DMA((_PLAN["nsem"],)),
        ],
        compiler_params=_compiler_params(),
    )(A_x.reshape(B, D), A_k_cache, A_v_cache, A_wq, A_wo, B_w1, B_b1, B_w2)
    return out.reshape(A_x.shape)
```
